```python
import jax
import jax.numpy as jnp

def _softmax(x, axis=-1):
    return jax.nn.softmax(x, axis=axis)
def _gelu(x):
    return jax.nn.gelu(x, approximate=True)
def _silu(x):
    return jax.nn.silu(x)
def _sigmoid(x):
    return jax.nn.sigmoid(x)
def _layernorm(x, axis=-1, eps=1e-5):
    m = jnp.mean(x, axis=axis, keepdims=True)
    v = jnp.var(x, axis=axis, keepdims=True)
    return (x - m) / jnp.sqrt(v + eps)
def _scatter_add(tgt, idx, src, axis=0):
    return tgt.at[idx].add(src)
def _segment_sum(src, seg, n):
    return jax.ops.segment_sum(src, seg, n)
class _Rng:
    def __init__(self, key):
        self._k = key
    def _next(self):
        self._k, sub = jax.random.split(self._k)
        return sub
    def normal(self, shape):
        return jax.random.normal(self._next(), shape, dtype=jnp.bfloat16)
    def randint(self, lo, hi, shape):
        return jax.random.randint(self._next(), shape, lo, hi, dtype=jnp.int32)
    def uniform(self, shape, lo=0.0, hi=1.0):
        return jax.random.uniform(self._next(), shape, jnp.bfloat16, lo, hi)
    def permutation(self, n):
        return jax.random.permutation(self._next(), n)


kernel_name = 'sequential_preLN__spectral_gfnet__swiglu_ffn__prompt'

def _fwd_setup_inputs():
    _rng = _Rng(jax.random.key(int.from_bytes(__import__("os").urandom(4), "little")))
    _w = (lambda a: (lambda t: t.astype(jnp.bfloat16) if jnp.issubdtype(t.dtype, jnp.floating) else t)(jnp.asarray(a)))
    def _A_setup():
        B, S, D = 1, 2048, 576
        Df = D // 2 + 1
        return {
            "x": _w((lambda *s: _rng.normal(s) * 0.05)(B, S, D)),
            "w_r": _w((lambda *s: _rng.normal(s) * 0.05)(S, Df) * 0.02),
            "w_i": _w((lambda *s: _rng.normal(s) * 0.05)(S, Df) * 0.02),
        }
    _A_in = _A_setup()

    def _B_setup():
        B, S, D, F = 1, 2048, 576, 4608
        return {
            "x": _w((lambda *s: _rng.normal(s) * 0.05)(B, S, D)),
            "w_gate": _w((lambda *s: _rng.normal(s) * 0.05)(D, F)),
            "w_up": _w((lambda *s: _rng.normal(s) * 0.05)(D, F)),
            "w_down": _w((lambda *s: _rng.normal(s) * 0.05)(F, D)),
        }
    _B_in = _B_setup()

    return {
        "A_x": _A_in["x"],
        "A_w_r": _A_in["w_r"],
        "A_w_i": _A_in["w_i"],
        "B_x": _B_in["x"],
        "B_w_gate": _B_in["w_gate"],
        "B_w_up": _B_in["w_up"],
        "B_w_down": _B_in["w_down"],
    }

def _fwd_reference(A_x, A_w_r, A_w_i, B_x, B_w_gate, B_w_up, B_w_down):
    def _A_ref(x, w_r, w_i):
        B, S, D = x.shape
        X = (lambda x, axes=(-2,-1): jnp.fft.rfft2(x.astype(jnp.float32), axes=axes))(x, axes=(-2, -1))
        W = w_r + 1j * w_i
        X = X * W
        y = (lambda x, s, axes=(-2,-1): jnp.fft.irfft2(x, s=s, axes=axes).astype(jnp.bfloat16))(X, (S, D), axes=(-2, -1))
        return y

    def _B_ref(x, w_gate, w_up, w_down):
        g = _silu(x @ w_gate)
        u = x @ w_up
        return (g * u) @ w_down

    x = A_x
    h = x + _A_ref(_layernorm(x, axis=-1), A_w_r, A_w_i)
    h2 = h + _B_ref(_layernorm(h, axis=-1), B_w_gate, B_w_up, B_w_down)
    return h2


def setup_inputs():
    _inp = _fwd_setup_inputs()
    _gk = jax.random.fold_in(jax.random.key(int.from_bytes(__import__("os").urandom(4), "little")), 2**31 - 1)
    _shapes = [[1, 2048, 576]]
    _dtypes = ['bfloat16']
    _gks = jax.random.split(_gk, len(_shapes))
    _gs = [jax.random.normal(k, s, dtype=jnp.dtype(d)) * 0.05 for k, s, d in zip(_gks, _shapes, _dtypes)]
    _inp["grad_out"] = _gs[0]
    return _inp

def reference(A_x, A_w_r, A_w_i, B_w_gate, B_w_up, B_w_down, B_x, grad_out):
    _const = dict(B_x=B_x)
    def _f(*_d):
        return _fwd_reference(**{'A_x': _d[0], 'A_w_r': _d[1], 'A_w_i': _d[2], 'B_w_gate': _d[3], 'B_w_up': _d[4], 'B_w_down': _d[5], **_const})
    _out, _vjp = jax.vjp(_f, A_x, A_w_r, A_w_i, B_w_gate, B_w_up, B_w_down)
    _grads = _vjp(grad_out)
    _out0 = jnp.asarray(_out)
    return (_out0, *[jnp.asarray(_g) for _g in _grads])
```

```python
import numpy as np
import jax
import jax.numpy as jnp
from jax import lax
from jax.experimental import pallas as pl
from jax.experimental.pallas import tpu as pltpu

S, D, F = 2048, 576, 4608
DF = D // 2 + 1
KR = 304
KP = 384
NLB = KP // 128
R1 = 16
R2 = 128
EPS = 1e-5
TF = 256
NF = F // TF
SU = 4
CU = 1
FC = 512
LC = 512
f32 = jnp.float32
bf16 = jnp.bfloat16
NT = (((1,), (1,)), ((), ()))
TN = (((0,), (0,)), ((), ()))


def _tables():
    d = np.arange(D)[:, None]
    k = np.arange(DF)[None, :]
    ang = 2.0 * np.pi * ((d * k) % D) / D
    cs, sn = np.cos(ang), -np.sin(ang)
    sn[:, 0] = 0.0
    sn[:, DF - 1] = 0.0
    cdi = np.zeros((D, 2 * KP), np.float64)
    cdi[:, :DF] = cs
    cdi[:, KP:KP + DF] = sn
    cdf = np.zeros((2 * KR, D), np.float64)
    cdf[:DF] = cs.T
    cdf[KR:KR + DF] = sn.T
    mf = np.zeros((R1, 2 * R2, 2 * R2), np.float64)
    j2 = np.arange(R2)[:, None]
    b = np.arange(R2)[None, :]
    for j1 in range(R1):
        a = 2.0 * np.pi * ((b * (j1 + R1 * j2)) % S) / S
        mr, mi_ = np.cos(a), -np.sin(a)
        mf[j1] = np.block([[mr, -mi_], [mi_, mr]])
    mi = np.ascontiguousarray(mf.transpose(0, 2, 1))
    cast = lambda t: jnp.asarray(t.astype(np.float32), dtype=bf16)
    return cast(cdf), cast(cdi), cast(mf), cast(mi)


def _cmul_const(z, k, n, sign):
    r, i = z
    k = k % n
    if k == 0:
        return r, i
    if 4 * k == n:
        return (-i, r) if sign > 0 else (i, -r)
    if 8 * k == n:
        c = float(np.sqrt(0.5))
        return ((r - i) * c, (r + i) * c) if sign > 0 else ((r + i) * c, (i - r) * c)
    if 8 * k == 3 * n:
        c = float(np.sqrt(0.5))
        return ((-r - i) * c, (r - i) * c) if sign > 0 else ((i - r) * c, (-r - i) * c)
    c = float(np.cos(2 * np.pi * k / n))
    s = float(sign * np.sin(2 * np.pi * k / n))
    return r * c - i * s, r * s + i * c


def _fft(xs, sign):
    n = len(xs)
    if n == 1:
        return xs
    ev = _fft(xs[0::2], sign)
    od = _fft(xs[1::2], sign)
    out = [None] * n
    for k in range(n // 2):
        tr, ti = _cmul_const(od[k], k, n, sign)
        out[k] = (ev[k][0] + tr, ev[k][1] + ti)
        out[k + n // 2] = (ev[k][0] - tr, ev[k][1] - ti)
    return out


def _ln_stats(v):
    mu = jnp.mean(v, axis=0, keepdims=True)
    vc = v - mu
    var = jnp.mean(vc * vc, axis=0, keepdims=True)
    rstd = lax.rsqrt(var + EPS)
    return vc * rstd, rstd


def _ln_bwd(dy, xhat, rstd):
    m1 = jnp.mean(dy, axis=0, keepdims=True)
    m2 = jnp.mean(dy * xhat, axis=0, keepdims=True)
    return (dy - m1 - xhat * m2) * rstd


def _kernel(x_hbm, wr_hbm, wi_hbm, go_hbm, wg_ref, wu_ref, wd_ref,
            cdf_hbm, cdi_hbm, mf_hbm, mi_hbm,
            h2_hbm, dx_hbm, dwr_hbm, dwi_hbm, dwg_ref, dwu_ref, dwd_ref,
            x_ref, wr_ref, wi_ref, go_ref, cdf_ref, cdi_ref, mf_ref, mi_ref,
            h2_ref, dx_ref, dwr_ref, dwi_ref,
            pt_s, vt_s, p_s, q_s, xs_s, wrs_s, wis_s, wt_s, ub_s, h_s, ln2_s,
            oacc_s, dacc_s, dwr_s, dwi_s, u1_s, rs_s, in_sem, cin_sem, out_sem):
    step = pl.program_id(0)
    nchunk = S // LC

    in_pairs = [(cdf_hbm, cdf_ref), (mf_hbm, mf_ref), (mi_hbm, mi_ref),
                (cdi_hbm, cdi_ref), (go_hbm, go_ref)]
    chunk_pairs = [(x_hbm, x_ref), (wr_hbm, wr_ref), (wi_hbm, wi_ref)]

    def in_copy(i):
        return pltpu.make_async_copy(in_pairs[i][0], in_pairs[i][1], in_sem.at[i])

    def chunk_copy(k, c):
        cols = pl.ds(pl.multiple_of(c * LC, LC), LC)
        return pltpu.make_async_copy(chunk_pairs[k][0].at[:, cols], chunk_pairs[k][1].at[:, cols],
                                     cin_sem.at[k, c])

    def out_copy(src, dst, c, k):
        cols = pl.ds(pl.multiple_of(c * LC, LC), LC)
        return pltpu.make_async_copy(src.at[:, cols], dst.at[:, cols], out_sem.at[k, c])

    def bfly_fwd():
        def body(rb, _):
            r0 = pl.multiple_of(rb * 8, 8)
            xs = [(pt_s[pl.ds(r0, 8), a * R2:(a + 1) * R2],
                   pt_s[pl.ds(KR + r0, 8), a * R2:(a + 1) * R2]) for a in range(R1)]
            ys = _fft(xs, -1)
            for j1 in range(R1):
                vt_s[pl.ds(r0, 8), 2 * R2 * j1:2 * R2 * j1 + R2] = ys[j1][0]
                vt_s[pl.ds(r0, 8), 2 * R2 * j1 + R2:2 * R2 * (j1 + 1)] = ys[j1][1]
            return 0
        lax.fori_loop(0, KR // 8, body, 0)

    def bfly_inv():
        def body(rb, _):
            r0 = pl.multiple_of(rb * 8, 8)
            for lb in range(NLB):
                l0 = lb * 128
                xs = [(q_s[j1, pl.ds(r0, 8), l0:l0 + 128],
                       q_s[j1, pl.ds(R2 + r0, 8), l0:l0 + 128]) for j1 in range(R1)]
                ys = _fft(xs, +1)
                for a in range(R1):
                    p_s[pl.ds(a * R2 + r0, 8), l0:l0 + 128] = ys[a][0]
                    p_s[pl.ds(a * R2 + r0, 8), KP + l0:KP + l0 + 128] = ys[a][1]
            return 0
        lax.fori_loop(0, R2 // 8, body, 0)

    def slab_spectrum(j1):
        cols = pl.ds(pl.multiple_of(j1 * 2 * R2, 2 * R2), 2 * R2)
        return lax.dot_general(mf_ref[j1], vt_s[:, cols].astype(bf16), NT,
                               preferred_element_type=f32)

    def load_w(j1):
        wr = jnp.concatenate([wrs_s[lb, pl.ds(j1, R2, stride=R1), :] for lb in range(NLB)], axis=1)
        wi = jnp.concatenate([wis_s[lb, pl.ds(j1, R2, stride=R1), :] for lb in range(NLB)], axis=1)
        return wr, wi

    @pl.when(step == 0)
    def _():
        in_copy(0).start()
        for c in range(2):
            for k in range(3):
                chunk_copy(k, c).start()
        kk = lax.broadcasted_iota(jnp.int32, (LC, KP), 1)
        scale = jnp.where((kk == 0) | (kk == DF - 1), 1.0, 2.0).astype(f32) * (1.0 / (S * D))
        vt_s[KR:KP, :] = jnp.zeros((KP - KR, 2 * S), f32)
        wt_s[:, DF - 1:KP, :] = jnp.zeros((2, KP - DF + 1, LC), f32)

        def pre(c, _):
            cols = pl.ds(pl.multiple_of(c * LC, LC), LC)
            for k in range(3):
                chunk_copy(k, c).wait()

            @pl.when(c + 2 < nchunk)
            def _():
                for k in range(3):
                    chunk_copy(k, c + 2).start()
            xh, rstd = _ln_stats(x_ref[:, cols].astype(f32))
            u = xh.astype(bf16)
            u1_s[:, cols] = u
            rs_s[0:1, cols] = rstd
            pt_s[:, cols] = jnp.dot(cdf_ref[...], u, preferred_element_type=f32)
            oacc_s[:, cols] = jnp.zeros((D, LC), f32)
            dacc_s[:, cols] = jnp.zeros((D, LC), f32)
            wt_s[0, 0:DF, :] = wr_ref[:, cols].astype(f32)
            wt_s[1, 0:DF, :] = wi_ref[:, cols].astype(f32)
            for i, dst in ((0, wrs_s), (1, wis_s)):
                w = wt_s[i].T * scale
                for lb in range(NLB):
                    dst[lb, cols, :] = w[:, lb * 128:(lb + 1) * 128]
            return 0
        with jax.named_scope("p1_wait"):
            in_copy(0).wait()
        in_copy(1).start()
        in_copy(2).start()
        with jax.named_scope("p1_pre"):
            lax.fori_loop(0, nchunk, pre, 0, unroll=CU)
        in_copy(3).start()
        in_copy(4).start()
        with jax.named_scope("p1_bf"):
            bfly_fwd()
        with jax.named_scope("p1_wait2"):
            in_copy(1).wait()
            in_copy(2).wait()

        def slab(jj, _):
            for u in range(SU):
                j1 = jj * SU + u
                xq = slab_spectrum(j1)
                xs_s[j1] = xq
                xr, xi = xq[:R2], xq[R2:]
                wr, wi = load_w(j1)
                z = jnp.concatenate([xr * wr - xi * wi, xr * wi + xi * wr], axis=0).astype(bf16)
                q_s[j1] = jnp.dot(mi_ref[j1], z, preferred_element_type=f32)
            return 0
        with jax.named_scope("p1_slab"):
            lax.fori_loop(0, R1 // SU, slab, 0)

        with jax.named_scope("p1_bi"):
            bfly_inv()
        in_copy(3).wait()

        def post(c, _):
            cols = pl.ds(pl.multiple_of(c * LC, LC), LC)
            y = lax.dot_general(cdi_ref[...], p_s[cols, :].astype(bf16), NT,
                                preferred_element_type=f32)
            h = (x_ref[:, cols].astype(f32) + y.astype(bf16).astype(f32)).astype(bf16)
            h_s[:, cols] = h
            xh, rstd = _ln_stats(h.astype(f32))
            ln2_s[:, cols] = xh.astype(bf16)
            rs_s[1:2, cols] = rstd
            return 0
        with jax.named_scope("p1_post"):
            lax.fori_loop(0, nchunk, post, 0, unroll=CU)
        in_copy(4).wait()

    with jax.named_scope("ffn"):
        ln2 = ln2_s[...]
        go = go_ref[...]
        wg = wg_ref[...]
        wu = wu_ref[...]
        wd = wd_ref[...]
        a = lax.dot_general(wg, ln2, TN, preferred_element_type=f32)
        b = lax.dot_general(wu, ln2, TN, preferred_element_type=f32)
        dm = lax.dot_general(wd, go, TN, preferred_element_type=f32)
        sig = jax.nn.sigmoid(a)
        g = a * sig
        m = (g * b).astype(bf16)
        db = (dm * g).astype(bf16)
        da = (dm * b * (sig * (1.0 + a * (1.0 - sig)))).astype(bf16)
        oacc_s[...] += jnp.dot(wd, m, preferred_element_type=f32)
        dwd_ref[...] = lax.dot_general(go, m, NT, preferred_element_type=f32).astype(bf16)
        dwg_ref[...] = lax.dot_general(ln2, da, NT, preferred_element_type=f32).astype(bf16)
        dwu_ref[...] = lax.dot_general(ln2, db, NT, preferred_element_type=f32).astype(bf16)
        dacc_s[...] += (jnp.dot(wg, da, preferred_element_type=f32)
                        + jnp.dot(wu, db, preferred_element_type=f32))

    @pl.when(step == NF - 1)
    def _():
        def pre(c, _):
            cols = pl.ds(pl.multiple_of(c * LC, LC), LC)
            h = h_s[:, cols].astype(f32)
            h2_ref[:, cols] = (h + oacc_s[:, cols]).astype(bf16)
            out_copy(h2_ref, h2_hbm, c, 0).start()
            dh = go_ref[:, cols].astype(f32) + _ln_bwd(dacc_s[:, cols], ln2_s[:, cols].astype(f32),
                                                       rs_s[1:2, cols])
            dh = dh.astype(bf16)
            ub_s[:, cols] = dh
            pt_s[:, cols] = jnp.dot(cdf_ref[...], dh, preferred_element_type=f32)
            return 0
        with jax.named_scope("p3_pre"):
            lax.fori_loop(0, nchunk, pre, 0, unroll=CU)
        with jax.named_scope("p3_bf"):
            bfly_fwd()

        kk = lax.broadcasted_iota(jnp.int32, (R2, KP), 1)
        scale = jnp.where((kk == 0) | (kk == DF - 1), 1.0, 2.0).astype(f32) * (1.0 / (S * D))

        def slab(jj, _):
            for u in range(SU):
                j1 = jj * SU + u
                gq = slab_spectrum(j1)
                gr, gi = gq[:R2], gq[R2:]
                xq = xs_s[j1]
                xr, xi = xq[:R2], xq[R2:]
                dwrv = (gr * xr + gi * xi) * scale
                dwiv = (gi * xr - gr * xi) * scale
                for lb in range(NLB):
                    dwr_s[lb, pl.ds(j1, R2, stride=R1), :] = dwrv[:, lb * 128:(lb + 1) * 128]
                    dwi_s[lb, pl.ds(j1, R2, stride=R1), :] = dwiv[:, lb * 128:(lb + 1) * 128]
                wr, wi = load_w(j1)
                z = jnp.concatenate([gr * wr + gi * wi, gi * wr - gr * wi], axis=0).astype(bf16)
                q_s[j1] = jnp.dot(mi_ref[j1], z, preferred_element_type=f32)
            return 0
        with jax.named_scope("p3_slab"):
            lax.fori_loop(0, R1 // SU, slab, 0)

        with jax.named_scope("p3_bi"):
            bfly_inv()

        def post(c, _):
            cols = pl.ds(pl.multiple_of(c * LC, LC), LC)
            du = lax.dot_general(cdi_ref[...], p_s[cols, :].astype(bf16), NT,
                                 preferred_element_type=f32)
            dx = ub_s[:, cols].astype(f32) + _ln_bwd(du, u1_s[:, cols].astype(f32), rs_s[0:1, cols])
            dx_ref[:, cols] = dx.astype(bf16)
            dwrv = jnp.concatenate([dwr_s[lb, cols, :] for lb in range(NLB)], axis=1).T
            dwiv = jnp.concatenate([dwi_s[lb, cols, :] for lb in range(NLB)], axis=1).T
            dwr_ref[:, cols] = dwrv[0:DF].astype(bf16)
            dwi_ref[:, cols] = dwiv[0:DF].astype(bf16)
            out_copy(dx_ref, dx_hbm, c, 1).start()
            out_copy(dwr_ref, dwr_hbm, c, 2).start()
            out_copy(dwi_ref, dwi_hbm, c, 3).start()
            return 0
        with jax.named_scope("p3_post"):
            lax.fori_loop(0, nchunk, post, 0, unroll=CU)

        def drain(c, _):
            out_copy(h2_ref, h2_hbm, c, 0).wait()
            out_copy(dx_ref, dx_hbm, c, 1).wait()
            out_copy(dwr_ref, dwr_hbm, c, 2).wait()
            out_copy(dwi_ref, dwi_hbm, c, 3).wait()
            return 0
        with jax.named_scope("p3_drain"):
            lax.fori_loop(0, nchunk, drain, 0)


@jax.jit
def pallas_sequential_preLN__spectral_gfnet__swiglu_ffn__prompt_kernel(
    A_x: jax.Array,
    A_w_r: jax.Array,
    A_w_i: jax.Array,
    B_x: jax.Array,
    B_w_gate: jax.Array,
    B_w_up: jax.Array,
    B_w_down: jax.Array,
    grad_out: jax.Array,
):
    del B_x
    xt = A_x.reshape(S, D).T
    got = grad_out.reshape(S, D).T
    wrt = A_w_r.T
    wit = A_w_i.T
    wdt = B_w_down.T
    cdf, cdi, mf, mi = _tables()

    wtile = pl.BlockSpec((D, TF), lambda i: (0, i))
    hbm = pl.BlockSpec(memory_space=pl.ANY)
    in_specs = [hbm, hbm, hbm, hbm, wtile, wtile, wtile, hbm, hbm, hbm, hbm]
    out_specs = [hbm, hbm, hbm, hbm, wtile, wtile, wtile]
    out_shape = [
        jax.ShapeDtypeStruct((D, S), bf16), jax.ShapeDtypeStruct((D, S), bf16),
        jax.ShapeDtypeStruct((DF, S), bf16), jax.ShapeDtypeStruct((DF, S), bf16),
        jax.ShapeDtypeStruct((D, F), bf16), jax.ShapeDtypeStruct((D, F), bf16),
        jax.ShapeDtypeStruct((D, F), bf16),
    ]
    scratch = [
        pltpu.VMEM((D, S), bf16),
        pltpu.VMEM((DF, S), bf16),
        pltpu.VMEM((DF, S), bf16),
        pltpu.VMEM((D, S), bf16),
        pltpu.VMEM((2 * KR, D), bf16),
        pltpu.VMEM((D, 2 * KP), bf16),
        pltpu.VMEM((R1, 2 * R2, 2 * R2), bf16),
        pltpu.VMEM((R1, 2 * R2, 2 * R2), bf16),
        pltpu.VMEM((D, S), bf16),
        pltpu.VMEM((D, S), bf16),
        pltpu.VMEM((DF, S), bf16),
        pltpu.VMEM((DF, S), bf16),
        pltpu.VMEM((2 * KR, S), f32),
        pltpu.VMEM((KP, 2 * S), f32),
        pltpu.VMEM((S, 2 * KP), f32),
        pltpu.VMEM((R1, 2 * R2, KP), f32),
        pltpu.VMEM((R1, 2 * R2, KP), f32),
        pltpu.VMEM((NLB, S, 128), f32),
        pltpu.VMEM((NLB, S, 128), f32),
        pltpu.VMEM((2, KP, LC), f32),
        pltpu.VMEM((D, S), bf16),
        pltpu.VMEM((D, S), bf16),
        pltpu.VMEM((D, S), bf16),
        pltpu.VMEM((D, S), f32),
        pltpu.VMEM((D, S), f32),
        pltpu.VMEM((NLB, S, 128), f32),
        pltpu.VMEM((NLB, S, 128), f32),
        pltpu.VMEM((D, S), bf16),
        pltpu.VMEM((8, S), f32),
        pltpu.SemaphoreType.DMA((5,)),
        pltpu.SemaphoreType.DMA((3, S // LC)),
        pltpu.SemaphoreType.DMA((4, S // LC)),
    ]
    h2, dx, dwr, dwi, dwg, dwu, dwd = pl.pallas_call(
        _kernel,
        grid=(NF,),
        in_specs=in_specs,
        out_specs=out_specs,
        out_shape=out_shape,
        scratch_shapes=scratch,
        compiler_params=pltpu.CompilerParams(
            dimension_semantics=("arbitrary",),
            vmem_limit_bytes=110 * 1024 * 1024,
        ),
    )(xt, wrt, wit, got, B_w_gate, B_w_up, wdt, cdf, cdi, mf, mi)
    return (h2.T.reshape(1, S, D), dx.T.reshape(1, S, D), dwr.T, dwi.T, dwg, dwu, dwd.T)
```

```python
import numpy as np
import jax
import jax.numpy as jnp
from jax import lax
from jax.experimental import pallas as pl
from jax.experimental.pallas import tpu as pltpu

S, D, F = 2048, 576, 4608
DF = D // 2 + 1
KR = 296
KP = 384
NLB = KP // 128
PK = 640
R1 = 16
R2 = 128
EPS = 1e-5
TF = 256
NF = F // TF
SU = 4
CU = 1
LC = 512
f32 = jnp.float32
bf16 = jnp.bfloat16
NT = (((1,), (1,)), ((), ()))
TN = (((0,), (0,)), ((), ()))


def _tables():
    d = np.arange(D)[:, None]
    k = np.arange(DF)[None, :]
    ang = 2.0 * np.pi * ((d * k) % D) / D
    cs, sn = np.cos(ang), -np.sin(ang)
    sn[:, 0] = 0.0
    sn[:, DF - 1] = 0.0
    cdi = np.zeros((D, PK), np.float64)
    cdi[:, 0:256] = cs[:, 0:256]
    cdi[:, 256:512] = sn[:, 0:256]
    cdi[:, 512:512 + DF - 256] = cs[:, 256:DF]
    cdi[:, 576:576 + DF - 256] = sn[:, 256:DF]
    cdf = np.zeros((2 * KR, D), np.float64)
    cdf[:DF] = cs.T
    cdf[KR:KR + DF] = sn.T
    mf = np.zeros((R1, 2 * R2, 2 * R2), np.float64)
    j2 = np.arange(R2)[:, None]
    b = np.arange(R2)[None, :]
    for j1 in range(R1):
        a = 2.0 * np.pi * ((b * (j1 + R1 * j2)) % S) / S
        mr, mi_ = np.cos(a), -np.sin(a)
        mf[j1] = np.block([[mr, -mi_], [mi_, mr]])
    mi = np.ascontiguousarray(mf.transpose(0, 2, 1))
    cast = lambda t: jnp.asarray(t.astype(np.float32), dtype=bf16)
    return cast(cdf), cast(cdi), cast(mf), cast(mi)


def _cmul_const(z, k, n, sign):
    r, i = z
    k = k % n
    if k == 0:
        return r, i
    if 4 * k == n:
        return (-i, r) if sign > 0 else (i, -r)
    if 8 * k == n:
        c = float(np.sqrt(0.5))
        return ((r - i) * c, (r + i) * c) if sign > 0 else ((r + i) * c, (i - r) * c)
    if 8 * k == 3 * n:
        c = float(np.sqrt(0.5))
        return ((-r - i) * c, (r - i) * c) if sign > 0 else ((i - r) * c, (-r - i) * c)
    c = float(np.cos(2 * np.pi * k / n))
    s = float(sign * np.sin(2 * np.pi * k / n))
    return r * c - i * s, r * s + i * c


def _fft(xs, sign):
    n = len(xs)
    if n == 1:
        return xs
    ev = _fft(xs[0::2], sign)
    od = _fft(xs[1::2], sign)
    out = [None] * n
    for k in range(n // 2):
        tr, ti = _cmul_const(od[k], k, n, sign)
        out[k] = (ev[k][0] + tr, ev[k][1] + ti)
        out[k + n // 2] = (ev[k][0] - tr, ev[k][1] - ti)
    return out


def _ln_stats(v):
    mu = jnp.mean(v, axis=0, keepdims=True)
    vc = v - mu
    var = jnp.mean(vc * vc, axis=0, keepdims=True)
    rstd = lax.rsqrt(var + EPS)
    return vc * rstd, rstd


def _ln_bwd(dy, xhat, rstd):
    m1 = jnp.mean(dy, axis=0, keepdims=True)
    m2 = jnp.mean(dy * xhat, axis=0, keepdims=True)
    return (dy - m1 - xhat * m2) * rstd


def _kernel(x_hbm, wr_hbm, wi_hbm, go_hbm, wg_ref, wu_ref, wd_ref,
            cdf_hbm, cdi_hbm, mf_hbm, mi_hbm,
            h2_hbm, dx_hbm, dwr_hbm, dwi_hbm, dwg_ref, dwu_ref, dwd_ref,
            x_ref, wr_ref, wi_ref, go_ref, cdf_ref, cdi_ref, mf_ref, mi_ref,
            h2_ref, dx_ref, dwr_ref, dwi_ref,
            pt_s, vt_s, p_s, q_s, xs_s, wrs_s, wis_s, wt_s, ub_s, h_s, ln2_s,
            oacc_s, dacc_s, dwr_s, dwi_s, u1_s, rs_s, in_sem, cin_sem, tab_sem, out_sem):
    step = pl.program_id(0)
    nchunk = S // LC

    in_pairs = [(cdf_hbm, cdf_ref), (cdi_hbm, cdi_ref), (go_hbm, go_ref)]
    tab_pairs = [(mf_hbm, mf_ref), (mi_hbm, mi_ref)]

    def tab_copy(k, g):
        rows = pl.ds(g * SU, SU)
        return pltpu.make_async_copy(tab_pairs[k][0].at[rows], tab_pairs[k][1].at[rows],
                                     tab_sem.at[k, g])
    chunk_pairs = [(x_hbm, x_ref), (wr_hbm, wr_ref), (wi_hbm, wi_ref)]

    def in_copy(i):
        return pltpu.make_async_copy(in_pairs[i][0], in_pairs[i][1], in_sem.at[i])

    def chunk_copy(k, c):
        cols = pl.ds(pl.multiple_of(c * LC, LC), LC)
        return pltpu.make_async_copy(chunk_pairs[k][0].at[:, cols], chunk_pairs[k][1].at[:, cols],
                                     cin_sem.at[k, c])

    def out_copy(src, dst, c, k):
        cols = pl.ds(pl.multiple_of(c * LC, LC), LC)
        return pltpu.make_async_copy(src.at[:, cols], dst.at[:, cols], out_sem.at[k, c])

    def bfly_fwd():
        def body(rb, _):
            r0 = pl.multiple_of(rb * 8, 8)
            xs = [(pt_s[pl.ds(r0, 8), a * R2:(a + 1) * R2],
                   pt_s[pl.ds(KR + r0, 8), a * R2:(a + 1) * R2]) for a in range(R1)]
            ys = _fft(xs, -1)
            for j1 in range(R1):
                vt_s[pl.ds(r0, 8), 2 * R2 * j1:2 * R2 * j1 + R2] = ys[j1][0]
                vt_s[pl.ds(r0, 8), 2 * R2 * j1 + R2:2 * R2 * (j1 + 1)] = ys[j1][1]
            return 0
        lax.fori_loop(0, KR // 8, body, 0)

    def bfly_inv():
        def body(rb, _):
            r0 = pl.multiple_of(rb * 8, 8)
            for lb in range(NLB):
                l0 = lb * 128
                xs = [(q_s[j1, pl.ds(r0, 8), l0:l0 + 128],
                       q_s[j1, pl.ds(R2 + r0, 8), l0:l0 + 128]) for j1 in range(R1)]
                ys = _fft(xs, +1)
                for a in range(R1):
                    if lb < 2:
                        p_s[pl.ds(a * R2 + r0, 8), l0:l0 + 128] = ys[a][0]
                        p_s[pl.ds(a * R2 + r0, 8), 256 + l0:256 + l0 + 128] = ys[a][1]
                    else:
                        p_s[pl.ds(a * R2 + r0, 8), 512:640] = (
                            ys[a][0] + pltpu.roll(ys[a][1], 64, 1))
            return 0
        lax.fori_loop(0, R2 // 8, body, 0)

    def slab_spectrum(j1):
        cols = pl.ds(pl.multiple_of(j1 * 2 * R2, 2 * R2), 2 * R2)
        return lax.dot_general(mf_ref[j1], vt_s[:, cols].astype(bf16), NT,
                               preferred_element_type=f32)

    def load_w(j1):
        wr = jnp.concatenate([wrs_s[lb, pl.ds(j1, R2, stride=R1), :] for lb in range(NLB)], axis=1)
        wi = jnp.concatenate([wis_s[lb, pl.ds(j1, R2, stride=R1), :] for lb in range(NLB)], axis=1)
        return wr, wi

    @pl.when(step == 0)
    def _():
        in_copy(0).start()
        for k in range(3):
            chunk_copy(k, 0).start()
        kk = lax.broadcasted_iota(jnp.int32, (LC, KP), 1)
        scale = jnp.where((kk == 0) | (kk == DF - 1), 1.0, 2.0).astype(f32) * (1.0 / (S * D))
        vt_s[KR:KP, :] = jnp.zeros((KP - KR, 2 * S), f32)
        wt_s[:, DF - 1:KP, :] = jnp.zeros((2, KP - DF + 1, LC), f32)

        def pre(c, _):
            cols = pl.ds(pl.multiple_of(c * LC, LC), LC)
            for k in range(3):
                chunk_copy(k, c).wait()

            @pl.when(c + 2 < nchunk)
            def _():
                for k in range(3):
                    chunk_copy(k, c + 2).start()

            @pl.when(c >= nchunk - 2)
            def _():
                for k in range(2):
                    tab_copy(k, c - (nchunk - 2)).start()
            xh, rstd = _ln_stats(x_ref[:, cols].astype(f32))
            u = xh.astype(bf16)
            u1_s[:, cols] = u
            rs_s[0:1, cols] = rstd
            pt_s[:, cols] = jnp.dot(cdf_ref[...], u, preferred_element_type=f32)
            oacc_s[:, cols] = jnp.zeros((D, LC), f32)
            dacc_s[:, cols] = jnp.zeros((D, LC), f32)
            wt_s[0, 0:DF, :] = wr_ref[:, cols].astype(f32)
            wt_s[1, 0:DF, :] = wi_ref[:, cols].astype(f32)
            for i, dst in ((0, wrs_s), (1, wis_s)):
                w = wt_s[i].T * scale
                for lb in range(NLB):
                    dst[lb, cols, :] = w[:, lb * 128:(lb + 1) * 128]
            return 0
        with jax.named_scope("p1_wait"):
            in_copy(0).wait()
        for k in range(3):
            chunk_copy(k, 1).start()
        with jax.named_scope("p1_pre"):
            lax.fori_loop(0, nchunk, pre, 0, unroll=CU)
        for g in range(2, R1 // SU):
            for k in range(2):
                tab_copy(k, g).start()
        with jax.named_scope("p1_bf"):
            bfly_fwd()
        in_copy(1).start()
        in_copy(2).start()

        def slab(jj, _):
            for k in range(2):
                tab_copy(k, jj).wait()
            for u in range(SU):
                j1 = jj * SU + u
                xq = slab_spectrum(j1)
                xs_s[j1] = xq
                xr, xi = xq[:R2], xq[R2:]
                wr, wi = load_w(j1)
                z = jnp.concatenate([xr * wr - xi * wi, xr * wi + xi * wr], axis=0).astype(bf16)
                q_s[j1] = jnp.dot(mi_ref[j1], z, preferred_element_type=f32)
            return 0
        with jax.named_scope("p1_slab"):
            lax.fori_loop(0, R1 // SU, slab, 0)

        with jax.named_scope("p1_bi"):
            bfly_inv()
        in_copy(1).wait()

        def post(c, _):
            cols = pl.ds(pl.multiple_of(c * LC, LC), LC)
            y = lax.dot_general(cdi_ref[...], p_s[cols, :].astype(bf16), NT,
                                preferred_element_type=f32)
            h = (x_ref[:, cols].astype(f32) + y.astype(bf16).astype(f32)).astype(bf16)
            h_s[:, cols] = h
            xh, rstd = _ln_stats(h.astype(f32))
            ln2_s[:, cols] = xh.astype(bf16)
            rs_s[1:2, cols] = rstd
            return 0
        with jax.named_scope("p1_post"):
            lax.fori_loop(0, nchunk, post, 0, unroll=CU)
        in_copy(2).wait()

    with jax.named_scope("ffn"):
        ln2 = ln2_s[...]
        go = go_ref[...]
        wg = wg_ref[...]
        wu = wu_ref[...]
        wd = wd_ref[...]
        a = lax.dot_general(wg, ln2, TN, preferred_element_type=f32)
        b = lax.dot_general(wu, ln2, TN, preferred_element_type=f32)
        dm = lax.dot_general(wd, go, TN, preferred_element_type=f32)
        sig = jax.nn.sigmoid(a)
        g = a * sig
        m = (g * b).astype(bf16)
        db = (dm * g).astype(bf16)
        da = (dm * b * (sig * (1.0 + a * (1.0 - sig)))).astype(bf16)
        oacc_s[...] += jnp.dot(wd, m, preferred_element_type=f32)
        dwd_ref[...] = lax.dot_general(go, m, NT, preferred_element_type=f32).astype(bf16)
        dwg_ref[...] = lax.dot_general(ln2, da, NT, preferred_element_type=f32).astype(bf16)
        dwu_ref[...] = lax.dot_general(ln2, db, NT, preferred_element_type=f32).astype(bf16)
        dacc_s[...] += (jnp.dot(wg, da, preferred_element_type=f32)
                        + jnp.dot(wu, db, preferred_element_type=f32))

    @pl.when(step == NF - 1)
    def _():
        def pre(c, _):
            cols = pl.ds(pl.multiple_of(c * LC, LC), LC)
            h = h_s[:, cols].astype(f32)
            h2_ref[:, cols] = (h + oacc_s[:, cols]).astype(bf16)
            out_copy(h2_ref, h2_hbm, c, 0).start()
            dh = go_ref[:, cols].astype(f32) + _ln_bwd(dacc_s[:, cols], ln2_s[:, cols].astype(f32),
                                                       rs_s[1:2, cols])
            dh = dh.astype(bf16)
            ub_s[:, cols] = dh
            pt_s[:, cols] = jnp.dot(cdf_ref[...], dh, preferred_element_type=f32)
            return 0
        with jax.named_scope("p3_pre"):
            lax.fori_loop(0, nchunk, pre, 0, unroll=CU)
        with jax.named_scope("p3_bf"):
            bfly_fwd()

        kk = lax.broadcasted_iota(jnp.int32, (R2, KP), 1)
        scale = jnp.where((kk == 0) | (kk == DF - 1), 1.0, 2.0).astype(f32) * (1.0 / (S * D))

        def slab(jj, _):
            for u in range(SU):
                j1 = jj * SU + u
                gq = slab_spectrum(j1)
                gr, gi = gq[:R2], gq[R2:]
                xq = xs_s[j1]
                xr, xi = xq[:R2], xq[R2:]
                dwrv = (gr * xr + gi * xi) * scale
                dwiv = (gi * xr - gr * xi) * scale
                for lb in range(NLB):
                    dwr_s[lb, pl.ds(j1, R2, stride=R1), :] = dwrv[:, lb * 128:(lb + 1) * 128]
                    dwi_s[lb, pl.ds(j1, R2, stride=R1), :] = dwiv[:, lb * 128:(lb + 1) * 128]
                wr, wi = load_w(j1)
                z = jnp.concatenate([gr * wr + gi * wi, gi * wr - gr * wi], axis=0).astype(bf16)
                q_s[j1] = jnp.dot(mi_ref[j1], z, preferred_element_type=f32)
            return 0
        with jax.named_scope("p3_slab"):
            lax.fori_loop(0, R1 // SU, slab, 0)

        with jax.named_scope("p3_bi"):
            bfly_inv()

        def post(c, _):
            cols = pl.ds(pl.multiple_of(c * LC, LC), LC)
            du = lax.dot_general(cdi_ref[...], p_s[cols, :].astype(bf16), NT,
                                 preferred_element_type=f32)
            dx = ub_s[:, cols].astype(f32) + _ln_bwd(du, u1_s[:, cols].astype(f32), rs_s[0:1, cols])
            dx_ref[:, cols] = dx.astype(bf16)
            dwrv = jnp.concatenate([dwr_s[lb, cols, :] for lb in range(NLB)], axis=1).T
            dwiv = jnp.concatenate([dwi_s[lb, cols, :] for lb in range(NLB)], axis=1).T
            dwr_ref[:, cols] = dwrv[0:DF].astype(bf16)
            dwi_ref[:, cols] = dwiv[0:DF].astype(bf16)
            out_copy(dx_ref, dx_hbm, c, 1).start()
            out_copy(dwr_ref, dwr_hbm, c, 2).start()
            out_copy(dwi_ref, dwi_hbm, c, 3).start()
            return 0
        with jax.named_scope("p3_post"):
            lax.fori_loop(0, nchunk, post, 0, unroll=CU)

        def drain(c, _):
            out_copy(h2_ref, h2_hbm, c, 0).wait()
            out_copy(dx_ref, dx_hbm, c, 1).wait()
            out_copy(dwr_ref, dwr_hbm, c, 2).wait()
            out_copy(dwi_ref, dwi_hbm, c, 3).wait()
            return 0
        with jax.named_scope("p3_drain"):
            lax.fori_loop(0, nchunk, drain, 0)


@jax.jit
def pallas_sequential_preLN__spectral_gfnet__swiglu_ffn__prompt_kernel(
    A_x: jax.Array,
    A_w_r: jax.Array,
    A_w_i: jax.Array,
    B_x: jax.Array,
    B_w_gate: jax.Array,
    B_w_up: jax.Array,
    B_w_down: jax.Array,
    grad_out: jax.Array,
):
    del B_x
    xt = A_x.reshape(S, D).T
    got = grad_out.reshape(S, D).T
    wrt = A_w_r.T
    wit = A_w_i.T
    wdt = B_w_down.T
    cdf, cdi, mf, mi = _tables()

    wtile = pl.BlockSpec((D, TF), lambda i: (0, i))
    hbm = pl.BlockSpec(memory_space=pl.ANY)
    in_specs = [hbm, hbm, hbm, hbm, wtile, wtile, wtile, hbm, hbm, hbm, hbm]
    out_specs = [hbm, hbm, hbm, hbm, wtile, wtile, wtile]
    out_shape = [
        jax.ShapeDtypeStruct((D, S), bf16), jax.ShapeDtypeStruct((D, S), bf16),
        jax.ShapeDtypeStruct((DF, S), bf16), jax.ShapeDtypeStruct((DF, S), bf16),
        jax.ShapeDtypeStruct((D, F), bf16), jax.ShapeDtypeStruct((D, F), bf16),
        jax.ShapeDtypeStruct((D, F), bf16),
    ]
    scratch = [
        pltpu.VMEM((D, S), bf16),
        pltpu.VMEM((DF, S), bf16),
        pltpu.VMEM((DF, S), bf16),
        pltpu.VMEM((D, S), bf16),
        pltpu.VMEM((2 * KR, D), bf16),
        pltpu.VMEM((D, PK), bf16),
        pltpu.VMEM((R1, 2 * R2, 2 * R2), bf16),
        pltpu.VMEM((R1, 2 * R2, 2 * R2), bf16),
        pltpu.VMEM((D, S), bf16),
        pltpu.VMEM((D, S), bf16),
        pltpu.VMEM((DF, S), bf16),
        pltpu.VMEM((DF, S), bf16),
        pltpu.VMEM((2 * KR, S), f32),
        pltpu.VMEM((KP, 2 * S), f32),
        pltpu.VMEM((S, PK), f32),
        pltpu.VMEM((R1, 2 * R2, KP), f32),
        pltpu.VMEM((R1, 2 * R2, KP), f32),
        pltpu.VMEM((NLB, S, 128), f32),
        pltpu.VMEM((NLB, S, 128), f32),
        pltpu.VMEM((2, KP, LC), f32),
        pltpu.VMEM((D, S), bf16),
        pltpu.VMEM((D, S), bf16),
        pltpu.VMEM((D, S), bf16),
        pltpu.VMEM((D, S), f32),
        pltpu.VMEM((D, S), f32),
        pltpu.VMEM((NLB, S, 128), f32),
        pltpu.VMEM((NLB, S, 128), f32),
        pltpu.VMEM((D, S), bf16),
        pltpu.VMEM((8, S), f32),
        pltpu.SemaphoreType.DMA((3,)),
        pltpu.SemaphoreType.DMA((3, S // LC)),
        pltpu.SemaphoreType.DMA((2, R1 // SU)),
        pltpu.SemaphoreType.DMA((4, S // LC)),
    ]
    h2, dx, dwr, dwi, dwg, dwu, dwd = pl.pallas_call(
        _kernel,
        grid=(NF,),
        in_specs=in_specs,
        out_specs=out_specs,
        out_shape=out_shape,
        scratch_shapes=scratch,
        compiler_params=pltpu.CompilerParams(
            dimension_semantics=("arbitrary",),
            vmem_limit_bytes=110 * 1024 * 1024,
        ),
    )(xt, wrt, wit, got, B_w_gate, B_w_up, wdt, cdf, cdi, mf, mi)
    return (h2.T.reshape(1, S, D), dx.T.reshape(1, S, D), dwr.T, dwi.T, dwg, dwu, dwd.T)
```
